```python
import jax
import jax.numpy as jnp

def _softmax(x, axis=-1):
    return jax.nn.softmax(x, axis=axis)
def _gelu(x):
    return jax.nn.gelu(x, approximate=True)
def _silu(x):
    return jax.nn.silu(x)
def _sigmoid(x):
    return jax.nn.sigmoid(x)
def _layernorm(x, axis=-1, eps=1e-5):
    m = jnp.mean(x, axis=axis, keepdims=True)
    v = jnp.var(x, axis=axis, keepdims=True)
    return (x - m) / jnp.sqrt(v + eps)
def _scatter_add(tgt, idx, src, axis=0):
    return tgt.at[idx].add(src)
def _segment_sum(src, seg, n):
    return jax.ops.segment_sum(src, seg, n)
class _Rng:
    def __init__(self, key):
        self._k = key
    def _next(self):
        self._k, sub = jax.random.split(self._k)
        return sub
    def normal(self, shape):
        return jax.random.normal(self._next(), shape, dtype=jnp.bfloat16)
    def randint(self, lo, hi, shape):
        return jax.random.randint(self._next(), shape, lo, hi, dtype=jnp.int32)
    def uniform(self, shape, lo=0.0, hi=1.0):
        return jax.random.uniform(self._next(), shape, jnp.bfloat16, lo, hi)
    def permutation(self, n):
        return jax.random.permutation(self._next(), n)


kernel_name = 'sequential_preLN__compressed_kv_cla__moe_arch_mod__prompt'

def setup_inputs():
    _rng = _Rng(jax.random.key(int.from_bytes(__import__("os").urandom(4), "little")))
    _w = (lambda a: (lambda t: t.astype(jnp.bfloat16) if jnp.issubdtype(t.dtype, jnp.floating) else t)(jnp.asarray(a)))
    def _A_setup():
        B, H, Sq, Sk, D, M = 1, 32, 2048, 2048, 128, 1024
        Dc = 4 * D
        return {
            "x": _w((lambda *s: _rng.normal(s) * 0.05)(B, Sq, M)),
            "c_kv": _w((lambda *s: _rng.normal(s) * 0.05)(B, Sk, Dc)),
            "w_q": _w((lambda *s: _rng.normal(s) * 0.05)(M, H, D) * (M ** -0.5)),
            "w_uk": _w((lambda *s: _rng.normal(s) * 0.05)(Dc, H, D) * (Dc ** -0.5)),
            "w_uv": _w((lambda *s: _rng.normal(s) * 0.05)(Dc, H, D) * (Dc ** -0.5)),
            "w_o": _w((lambda *s: _rng.normal(s) * 0.05)(H, D, M) * ((H * D) ** -0.5)),
        }
    _A_in = _A_setup()

    def _B_setup():
        B, S, D, F, C = 1, 2048, 1024, 3584, 2
        return {
            "x": _w((lambda *s: _rng.normal(s) * 0.05)(B, S, D)),
            "w_r": _w((lambda *s: _rng.normal(s) * 0.05)(D)),
            "w_gate": _w((lambda *s: _rng.normal(s) * 0.05)(D, F)),
            "w_up": _w((lambda *s: _rng.normal(s) * 0.05)(D, F)),
            "w_down": _w((lambda *s: _rng.normal(s) * 0.05)(F, D)),
        }
    _B_in = _B_setup()

    return {
        "A_x": _A_in["x"],
        "A_c_kv": _A_in["c_kv"],
        "A_w_q": _A_in["w_q"],
        "A_w_uk": _A_in["w_uk"],
        "A_w_uv": _A_in["w_uv"],
        "A_w_o": _A_in["w_o"],
        "B_x": _B_in["x"],
        "B_w_r": _B_in["w_r"],
        "B_w_gate": _B_in["w_gate"],
        "B_w_up": _B_in["w_up"],
        "B_w_down": _B_in["w_down"],
    }

def reference(A_x, A_c_kv, A_w_q, A_w_uk, A_w_uv, A_w_o, B_x, B_w_r, B_w_gate, B_w_up, B_w_down):
    def _A_ref(x, c_kv, w_q, w_uk, w_uv, w_o):
        B, Sq, M = x.shape[0], x.shape[1], x.shape[2]
        Sk = c_kv.shape[1]
        H, D = w_q.shape[1], w_q.shape[2]
        q = jnp.einsum("bqm,mhd->bhqd", x, w_q)
        k = jnp.einsum("bkc,chd->bhkd", c_kv, w_uk)
        v = jnp.einsum("bkc,chd->bhkd", c_kv, w_uv)
        scores = jnp.einsum("bhqd,bhkd->bhqk", q, k) * (D ** -0.5)
        off = Sk - Sq
        qi = jnp.arange(Sq)[:, None]
        kj = jnp.arange(Sk)[None, :]
        cmask = kj <= (qi + off)
        scores = jnp.where(cmask[None, None], scores, -1e9)
        p = _softmax(scores, axis=-1)
        ctx = jnp.einsum("bhqk,bhkd->bhqd", p, v)
        return jnp.einsum("bhqd,hdm->bqm", ctx, w_o)

    def _B_ref(x, w_r, w_gate, w_up, w_down):
        B, S, D = x.shape
        C = 2
        r = x @ w_r
        idx = jnp.argsort(-r, axis=-1)[:, :C]
        idx_e = jnp.repeat(idx.reshape(B, C, 1), D, axis=2)
        x_sel = jnp.take_along_axis(x, idx_e, axis=1)
        g = _silu(x_sel @ w_gate)
        u = x_sel @ w_up
        y = (g * u) @ w_down
        r_sel = _sigmoid(jnp.take_along_axis(r, idx, axis=1))
        y = y * r_sel.reshape(B, C, 1)
        b_off = (jnp.arange(B) * S).reshape(B, 1)
        flat_idx = (idx + b_off).reshape(B * C)
        zero = (x * 0.0).reshape(B * S, D)
        upd = _scatter_add(zero, flat_idx, y.reshape(B * C, D), axis=0)
        return x + upd.reshape(B, S, D)

    x = A_x
    h = x + _A_ref(_layernorm(x, axis=-1), A_c_kv, A_w_q, A_w_uk, A_w_uv, A_w_o)
    h2 = h + _B_ref(_layernorm(h, axis=-1), B_w_r, B_w_gate, B_w_up, B_w_down)
    return h2
```

```python
import functools
import math

import numpy as np
import jax
import jax.numpy as jnp
from jax import lax
import jax.experimental.pallas as pl
import jax.experimental.pallas.tpu as pltpu

S = 2048
M = 1024
H = 32
D = 128
DC = 512
F = 3584
EPS = 1e-5
BQ = 256
DEP = False
PSTART = 15
PR = 2048
RBS = (1024, 512, 256, 256)
NEG = -1e30
QSCALE = float(D ** -0.5 * math.log2(math.e))

f32 = jnp.float32
bf16 = jnp.bfloat16
u32 = jnp.uint32


def _ln(x):
    m = jnp.mean(x, axis=-1, keepdims=True)
    xc = x - m
    v = jnp.mean(xc * xc, axis=-1, keepdims=True)
    return xc * lax.rsqrt(v + EPS)


def _unpack_pair(raw32, base, g4, o, rows):
    w = raw32.at[pl.ds(base + g4, rows * (H // 2) - 12), :][pl.ds(o, rows, stride=H // 2), :]
    lo = lax.bitcast_convert_type(w.astype(jnp.uint16), bf16)
    hi = lax.bitcast_convert_type((w >> 16).astype(jnp.uint16), bf16)
    return jnp.concatenate([lo, hi], axis=1)


def _softmax_rows(s):
    m = jnp.max(s, axis=1, keepdims=True)
    p = jnp.exp2(s - m)
    l = jnp.sum(p, axis=1, keepdims=True)
    rl = pl.reciprocal(l, approx=True)
    rl = rl * (2.0 - l * rl)
    return p.astype(bf16), rl


T = BQ // 2


def _scores(q_ref, k_ref, a, i):
    lanes = pl.ds(a * D, D)
    L = (i + 1) * BQ
    nt = (((1,), (1,)), ((), ()))
    q = q_ref[pl.ds(i * BQ, BQ), lanes]
    s = lax.dot_general(q, k_ref[pl.ds(0, L - T), lanes], nt, preferred_element_type=f32)
    s_last = lax.dot_general(q[T:], k_ref[pl.ds(L - T, T), lanes], nt, preferred_element_type=f32)
    return s, s_last


def _probs(s, s_last, i):
    row = lax.broadcasted_iota(jnp.int32, (T, T), 0)
    col = lax.broadcasted_iota(jnp.int32, (T, T), 1)
    tri = col <= row
    L = (i + 1) * BQ
    sd = jnp.where(tri, s[:T, L - BQ:], NEG)
    s_top = jnp.concatenate([s[:T, :L - BQ], sd], axis=1) if i > 0 else sd
    s_bot = jnp.concatenate([s[T:], jnp.where(tri, s_last, NEG)], axis=1)
    p_top, rl_top = _softmax_rows(s_top)
    p_bot, rl_bot = _softmax_rows(s_bot)
    p = jnp.concatenate([p_top, p_bot[:, :L - T]], axis=0)
    return p, p_bot[:, L - T:], rl_top, rl_bot


def _context(pr, v_ref, ctx_ref, a, i, h0):
    p, p_last, rl_top, rl_bot = pr
    lanes = pl.ds(a * D, D)
    L = (i + 1) * BQ
    o = jnp.dot(p, v_ref[pl.ds(0, L - T), lanes], preferred_element_type=f32)
    o_last = jnp.dot(p_last, v_ref[pl.ds(L - T, T), lanes], preferred_element_type=f32)
    o = jnp.concatenate([o[:T] * rl_top, (o[T:] + o_last) * rl_bot], axis=0)
    ctx_ref[pl.ds(pl.multiple_of((h0 + a) * S + i * BQ, BQ), BQ), :] = o.astype(bf16)


def _attention_phase(x_hbm, ckv_hbm, wq_hbm, wuk_hbm, wuv_hbm, c_wo, x_v, xn_v, ctx_v, sems,
                     ckv_v, wq_v, wk_v, wv_v, q_v, k_v, v_v):
    nq, nk = M * H, DC * H
    c_x = pltpu.make_async_copy(x_hbm, x_v, sems.at[0])
    c_ckv = pltpu.make_async_copy(ckv_hbm, ckv_v, sems.at[1])
    c_wq = pltpu.make_async_copy(wq_hbm, ctx_v.at[pl.ds(0, nq), :], sems.at[2])
    c_wuk = pltpu.make_async_copy(wuk_hbm, ctx_v.at[pl.ds(nq, nk), :], sems.at[3])
    c_wuv = pltpu.make_async_copy(wuv_hbm, ctx_v.at[pl.ds(nq + nk, nk), :], sems.at[4])
    raw32 = ctx_v.bitcast(u32)

    def unpack(dst, base, rows):
        def body(g, _):
            g4 = pl.multiple_of(g * 4, 4)
            for o in range(4):
                dst[g4 + o] = _unpack_pair(raw32, base, g4, o, rows)
            return 0
        lax.fori_loop(0, H // 8, body, 0)

    def proj_kv(j):
        ckv = ckv_v[...]
        k_v[...] = jnp.dot(ckv, wk_v[j], preferred_element_type=f32).astype(bf16)
        v_v[...] = jnp.dot(ckv, wv_v[j], preferred_element_type=f32).astype(bf16)

    def proj_q(j):
        q_v[...] = (jnp.dot(xn_v[...], wq_v[j], preferred_element_type=f32) * QSCALE).astype(bf16)

    def attend(j):
        blocks = [(i, a) for i in reversed(range(S // BQ)) for a in range(2)]
        sc = _scores(q_v, k_v, blocks[0][1], blocks[0][0])
        for n, (i, a) in enumerate(blocks):
            nxt = _scores(q_v, k_v, blocks[n + 1][1], blocks[n + 1][0]) if n + 1 < len(blocks) else None
            _context(_probs(*sc, i), v_v, ctx_v, a, i, 2 * j)
            sc = nxt

    c_wq.start()
    c_x.start()
    c_wuk.start()
    c_wuv.start()
    c_ckv.start()
    c_wo.start()

    def ln_body(i, _):
        rows = pl.ds(pl.multiple_of(i * 256, 256), 256)
        xn_v[rows, :] = _ln(x_v[rows, :].astype(f32)).astype(bf16)
        return 0
    with jax.named_scope("wait_q"):
        c_wq.wait()
    with jax.named_scope("unpack_q"):
        unpack(wq_v, 0, M)
    with jax.named_scope("wait_x"):
        c_x.wait()
    with jax.named_scope("ln"):
        lax.fori_loop(0, S // 256, ln_body, 0)
    with jax.named_scope("proj_q0"):
        proj_q(0)
    with jax.named_scope("wait_k"):
        c_wuk.wait()
    with jax.named_scope("unpack_k"):
        unpack(wk_v, nq // 2, DC)
    with jax.named_scope("wait_v"):
        c_wuv.wait()
    with jax.named_scope("unpack_v"):
        unpack(wv_v, (nq + nk) // 2, DC)
    with jax.named_scope("proj_kv0"):
        c_ckv.wait()
        proj_kv(0)

    def pair_body(j, _):
        attend(j)
        proj_kv(j + 1)
        proj_q(j + 1)
        return 0
    with jax.named_scope("pairs"):
        lax.fori_loop(0, H // 2 - 1, pair_body, 0)
    with jax.named_scope("last_pair"):
        attend(H // 2 - 1)


def _tail_phase(wg_hbm, wu_hbm, wd_hbm, wr_ref, out_hbm, c_wo, x_v, xn_v, wo_v, ctx_v, idx_s, sems,
                wg_v, wu_v, wd_v, h_v, acc_v):
    c_wg = pltpu.make_async_copy(wg_hbm, wg_v, sems.at[6])
    c_wu = pltpu.make_async_copy(wu_hbm, wu_v, sems.at[7])
    c_wd = pltpu.make_async_copy(wd_hbm, wd_v, sems.at[8])
    c_wg.start()
    c_wu.start()
    c_wd.start()
    c_wo.wait()
    wr = wr_ref[...].astype(f32)

    def out_copy(start, size, sem):
        rows = pl.ds(start, size)
        return pltpu.make_async_copy(x_v.at[rows, :], out_hbm.at[rows, :], sems.at[sem])

    def project(start, RB):
        ctx = jnp.concatenate([ctx_v[pl.ds(hh * S + start, RB), :] for hh in range(H)], axis=1)
        acc_v[pl.ds(0, RB), :] = jnp.dot(ctx, wo_v[...], preferred_element_type=f32)

    def epilogue(start, RB, top):
        rows = pl.ds(start, RB)
        h = (x_v[rows, :].astype(f32) + acc_v[pl.ds(0, RB), :].astype(bf16).astype(f32)).astype(bf16)
        hf = h.astype(f32)
        ln = _ln(hf).astype(bf16)
        lnf = ln.astype(f32)
        r = jnp.sum(lnf * wr, axis=1, keepdims=True).astype(bf16).astype(f32)
        xn_v[rows, :] = ln
        x_v[rows, :] = (hf + lnf).astype(bf16)
        h_v[rows, :] = h
        out_copy(start, RB, 9).start()
        m1, i1, m2, i2 = top
        sub = lax.broadcasted_iota(jnp.int32, (8, 128), 0)
        for t in range(RB // 8):
            v = jnp.broadcast_to(r[t * 8:(t + 1) * 8], (8, 128))
            tok = sub + (start + t * 8)
            gt1 = v > m1
            gt2 = v > m2
            m2 = jnp.where(gt1, m1, jnp.where(gt2, v, m2))
            i2 = jnp.where(gt1, i1, jnp.where(gt2, tok, i2))
            m1 = jnp.where(gt1, v, m1)
            i1 = jnp.where(gt1, tok, i1)
        return m1, i1, m2, i2

    blocks = [(sum(RBS[:n]), RB) for n, RB in enumerate(RBS)]
    with jax.named_scope("out_proj"):
        ninf = jnp.full((8, 128), -jnp.inf, f32)
        zero = jnp.zeros((8, 128), jnp.int32)
        top = (ninf, zero, ninf, zero)
        project(*blocks[0])
        for n, blk in enumerate(blocks):
            top = epilogue(*blk, top)
            if n + 1 < len(blocks):
                project(*blocks[n + 1])

    r = jnp.concatenate([top[0], top[2]], axis=0)
    tok = jnp.concatenate([top[1], top[3]], axis=0)
    m1 = jnp.max(r, axis=0, keepdims=True)
    i1 = jnp.min(jnp.where(r == m1, tok, S - 1), axis=0, keepdims=True)
    r2 = jnp.where(tok == i1, -jnp.inf, r)
    m2 = jnp.max(r2, axis=0, keepdims=True)
    i2 = jnp.min(jnp.where(r2 == m2, tok, S - 1), axis=0, keepdims=True)
    idx_s[0] = jnp.max(i1)
    idx_s[1] = jnp.max(i2)
    m1 = m1[:, :1]
    m2 = m2[:, :1]
    t1 = idx_s[0]
    t2 = idx_s[1]
    b1 = pl.multiple_of((t1 // 16) * 16, 16)
    b2 = pl.multiple_of((t2 // 16) * 16, 16)
    sub = lax.broadcasted_iota(jnp.int32, (16, M), 0)
    sel1 = sub == (t1 - b1)
    sel2 = sub == (t2 - b2)
    ln1 = jnp.where(sel1, xn_v[pl.ds(b1, 16), :].astype(f32), 0.0)
    ln2 = jnp.where(sel2, xn_v[pl.ds(b2, 16), :].astype(f32), 0.0)
    x1 = jnp.sum(ln1, axis=0, keepdims=True)
    x2 = jnp.sum(ln2, axis=0, keepdims=True)
    xs = jnp.where(sub == 0, x1, jnp.where(sub == 1, x2, 0.0)).astype(bf16)

    c_wg.wait()
    c_wu.wait()
    g = jnp.dot(xs, wg_v[...], preferred_element_type=f32).astype(bf16).astype(f32)
    u = jnp.dot(xs, wu_v[...], preferred_element_type=f32).astype(bf16).astype(f32)
    sg = (g * (1.0 / (1.0 + jnp.exp(-g)))).astype(bf16).astype(f32)
    act = (sg * u).astype(bf16)
    with jax.named_scope("wait_wd"):
        c_wd.wait()
    y = jnp.dot(act, wd_v[...], preferred_element_type=f32).astype(bf16).astype(f32)
    g1 = (1.0 / (1.0 + jnp.exp(-m1))).astype(bf16).astype(f32)
    g2 = (1.0 / (1.0 + jnp.exp(-m2))).astype(bf16).astype(f32)
    y1 = (y[0:1, :] * g1).astype(bf16).astype(f32)
    y2 = (y[1:2, :] * g2).astype(bf16).astype(f32)

    with jax.named_scope("wait_out"):
        for blk in blocks:
            out_copy(*blk, 9).wait()
    for b, sel, yy in ((b1, sel1, y1), (b2, sel2, y2)):
        rows = pl.ds(b, 16)
        hrow = h_v[rows, :].astype(f32)
        lnrow = xn_v[rows, :].astype(f32)
        new = (hrow + (lnrow + yy).astype(bf16).astype(f32)).astype(bf16)
        x_v[rows, :] = jnp.where(sel, new, x_v[rows, :])

    out_copy(b1, 16, 9).start()

    @pl.when(b1 != b2)
    def _():
        c = out_copy(b2, 16, 0)
        c.start()
        c.wait()
    out_copy(b1, 16, 9).wait()


def _kernel(x_hbm, ckv_hbm, wq_hbm, wuk_hbm, wuv_hbm, wo_hbm, wr_ref, wg_hbm, wu_hbm, wd_hbm,
            out_hbm, x_v, xn_v, wo_v, ctx_v, idx_s, sems):
    c_wo = pltpu.make_async_copy(wo_hbm, wo_v, sems.at[5])
    pl.run_scoped(
        functools.partial(_attention_phase, x_hbm, ckv_hbm, wq_hbm, wuk_hbm, wuv_hbm, c_wo,
                          x_v, xn_v, ctx_v, sems),
        pltpu.VMEM((S, DC), bf16),
        pltpu.VMEM((H // 2, M, 2 * D), bf16), pltpu.VMEM((H // 2, DC, 2 * D), bf16),
        pltpu.VMEM((H // 2, DC, 2 * D), bf16),
        pltpu.VMEM((S, 2 * D), bf16), pltpu.VMEM((S, 2 * D), bf16), pltpu.VMEM((S, 2 * D), bf16))
    pl.run_scoped(
        functools.partial(_tail_phase, wg_hbm, wu_hbm, wd_hbm, wr_ref, out_hbm, c_wo,
                          x_v, xn_v, wo_v, ctx_v, idx_s, sems),
        pltpu.VMEM((M, F), bf16), pltpu.VMEM((M, F), bf16), pltpu.VMEM((F, M), bf16), pltpu.VMEM((S, M), bf16),
        pltpu.VMEM((max(RBS), M), f32))


@jax.jit
def pallas_sequential_preLN__compressed_kv_cla__moe_arch_mod__prompt_kernel(
    A_x, A_c_kv, A_w_q, A_w_uk, A_w_uv, A_w_o, B_x, B_w_r, B_w_gate, B_w_up, B_w_down,
):
    any_spec = pl.BlockSpec(memory_space=pl.ANY)
    vm = lambda shape, dt=bf16: pltpu.VMEM(shape, dt)
    out = pl.pallas_call(
        _kernel,
        out_shape=jax.ShapeDtypeStruct((S, M), bf16),
        in_specs=[any_spec] * 6 + [pl.BlockSpec(memory_space=pltpu.VMEM)] + [any_spec] * 3,
        out_specs=any_spec,
        scratch_shapes=[
            vm((S, M)), vm((S, M)), vm((H * D, M)), vm((S * H, D)),
            pltpu.SMEM((2,), jnp.int32),
            pltpu.SemaphoreType.DMA((10,)),
        ],
        compiler_params=pltpu.CompilerParams(vmem_limit_bytes=127 * 1024 * 1024),
    )(
        A_x.reshape(S, M), A_c_kv.reshape(S, DC),
        A_w_q.reshape(M * H, D), A_w_uk.reshape(DC * H, D), A_w_uv.reshape(DC * H, D),
        A_w_o.reshape(H * D, M), B_w_r.reshape(1, M), B_w_gate, B_w_up, B_w_down,
    )
    return out.reshape(1, S, M)
```

```python
import functools
import math

import numpy as np
import jax
import jax.numpy as jnp
from jax import lax
import jax.experimental.pallas as pl
import jax.experimental.pallas.tpu as pltpu

S = 2048
M = 1024
H = 32
D = 128
DC = 512
F = 3584
EPS = 1e-5
BQ = 256
LOOK = 2
DEP = False
PSTART = 15
PR = 2048
RBS = (1024, 512, 256, 256)
NEG = -1e30
QSCALE = float(D ** -0.5 * math.log2(math.e))

f32 = jnp.float32
bf16 = jnp.bfloat16
u32 = jnp.uint32


def _ln(x):
    m = jnp.mean(x, axis=-1, keepdims=True)
    xc = x - m
    v = jnp.mean(xc * xc, axis=-1, keepdims=True)
    return xc * lax.rsqrt(v + EPS)


def _unpack_pair(raw32, base, g4, o, rows):
    w = raw32.at[pl.ds(base + g4, rows * (H // 2) - 12), :][pl.ds(o, rows, stride=H // 2), :]
    lo = lax.bitcast_convert_type(w.astype(jnp.uint16), bf16)
    hi = lax.bitcast_convert_type((w >> 16).astype(jnp.uint16), bf16)
    return jnp.concatenate([lo, hi], axis=1)


def _softmax_rows(s):
    m = jnp.max(s, axis=1, keepdims=True)
    p = jnp.exp2(s - m)
    l = jnp.sum(p, axis=1, keepdims=True)
    rl = pl.reciprocal(l, approx=True)
    rl = rl * (2.0 - l * rl)
    return p.astype(bf16), rl


T = 128
NS = BQ // T


def _scores(q_ref, k_ref, a, i):
    lanes = pl.ds(a * D, D)
    k0 = i * BQ + T
    nt = (((1,), (1,)), ((), ()))
    q = q_ref[pl.ds(i * BQ, BQ), lanes]
    out = [lax.dot_general(q, k_ref[pl.ds(0, k0), lanes], nt, preferred_element_type=f32)]
    for t in range(1, NS):
        out.append(lax.dot_general(q[t * T:], k_ref[pl.ds(k0 + (t - 1) * T, T), lanes], nt,
                                   preferred_element_type=f32))
    return out


def _probs(sc, i):
    row = lax.broadcasted_iota(jnp.int32, (T, T), 0)
    col = lax.broadcasted_iota(jnp.int32, (T, T), 1)
    tri = col <= row
    k0 = i * BQ + T
    ps, rls = [], []
    for r in range(NS):
        parts = [sc[0][r * T:(r + 1) * T]] + [sc[t][(r - t) * T:(r - t + 1) * T] for t in range(1, r + 1)]
        s = jnp.concatenate(parts, axis=1) if len(parts) > 1 else parts[0]
        n = s.shape[1]
        sd = jnp.where(tri, s[:, n - T:], NEG)
        s = jnp.concatenate([s[:, :n - T], sd], axis=1) if n > T else sd
        p, rl = _softmax_rows(s)
        ps.append(p)
        rls.append(rl)
    pieces = [jnp.concatenate([p[:, :k0] for p in ps], axis=0) if NS > 1 else ps[0]]
    for t in range(1, NS):
        c = k0 + (t - 1) * T
        tiles = [ps[r][:, c:c + T] for r in range(t, NS)]
        pieces.append(jnp.concatenate(tiles, axis=0) if len(tiles) > 1 else tiles[0])
    return pieces, rls


def _context(pr, v_ref, ctx_ref, a, i, h0):
    pieces, rls = pr
    lanes = pl.ds(a * D, D)
    k0 = i * BQ + T
    o = jnp.dot(pieces[0], v_ref[pl.ds(0, k0), lanes], preferred_element_type=f32)
    strips = [o[r * T:(r + 1) * T] for r in range(NS)]
    for t in range(1, NS):
        ot = jnp.dot(pieces[t], v_ref[pl.ds(k0 + (t - 1) * T, T), lanes], preferred_element_type=f32)
        for r in range(t, NS):
            strips[r] = strips[r] + ot[(r - t) * T:(r - t + 1) * T]
    o = jnp.concatenate([strips[r] * rls[r] for r in range(NS)], axis=0)
    ctx_ref[pl.ds(pl.multiple_of((h0 + a) * S + i * BQ, BQ), BQ), :] = o.astype(bf16)


def _attention_phase(x_hbm, ckv_hbm, wq_hbm, wuk_hbm, wuv_hbm, c_wo, x_v, xn_v, ctx_v, sems,
                     ckv_v, wq_v, wk_v, wv_v, q_v, k_v, v_v):
    nq, nk = M * H, DC * H
    c_x = pltpu.make_async_copy(x_hbm, x_v, sems.at[0])
    c_ckv = pltpu.make_async_copy(ckv_hbm, ckv_v, sems.at[1])
    c_wq = pltpu.make_async_copy(wq_hbm, ctx_v.at[pl.ds(0, nq), :], sems.at[2])
    c_wuk = pltpu.make_async_copy(wuk_hbm, ctx_v.at[pl.ds(nq, nk), :], sems.at[3])
    c_wuv = pltpu.make_async_copy(wuv_hbm, ctx_v.at[pl.ds(nq + nk, nk), :], sems.at[4])
    raw32 = ctx_v.bitcast(u32)

    def unpack(dst, base, rows):
        def body(g, _):
            g4 = pl.multiple_of(g * 4, 4)
            for o in range(4):
                dst[g4 + o] = _unpack_pair(raw32, base, g4, o, rows)
            return 0
        lax.fori_loop(0, H // 8, body, 0)

    def proj_kv(j):
        ckv = ckv_v[...]
        k_v[...] = jnp.dot(ckv, wk_v[j], preferred_element_type=f32).astype(bf16)
        v_v[...] = jnp.dot(ckv, wv_v[j], preferred_element_type=f32).astype(bf16)

    def proj_q(j):
        q_v[...] = (jnp.dot(xn_v[...], wq_v[j], preferred_element_type=f32) * QSCALE).astype(bf16)

    def attend(j):
        blocks = [(i, a) for a in range(2) for i in reversed(range(S // BQ))]
        sc = [_scores(q_v, k_v, a, i) for i, a in blocks[:LOOK]]
        for n, (i, a) in enumerate(blocks):
            if n + LOOK < len(blocks):
                sc.append(_scores(q_v, k_v, blocks[n + LOOK][1], blocks[n + LOOK][0]))
            _context(_probs(sc.pop(0), i), v_v, ctx_v, a, i, 2 * j)

    c_wq.start()
    c_x.start()
    c_wuk.start()
    c_wuv.start()
    c_ckv.start()
    c_wo.start()

    def ln_body(i, _):
        rows = pl.ds(pl.multiple_of(i * 256, 256), 256)
        xn_v[rows, :] = _ln(x_v[rows, :].astype(f32)).astype(bf16)
        return 0
    with jax.named_scope("wait_q"):
        c_wq.wait()
    with jax.named_scope("unpack_q"):
        unpack(wq_v, 0, M)
    with jax.named_scope("wait_x"):
        c_x.wait()
    with jax.named_scope("ln"):
        lax.fori_loop(0, S // 256, ln_body, 0)
    with jax.named_scope("proj_q0"):
        proj_q(0)
    with jax.named_scope("wait_k"):
        c_wuk.wait()
    with jax.named_scope("unpack_k"):
        unpack(wk_v, nq // 2, DC)
    with jax.named_scope("wait_v"):
        c_wuv.wait()
    with jax.named_scope("unpack_v"):
        unpack(wv_v, (nq + nk) // 2, DC)
    with jax.named_scope("proj_kv0"):
        c_ckv.wait()
        proj_kv(0)

    def pair_body(j, _):
        attend(j)
        proj_kv(j + 1)
        proj_q(j + 1)
        return 0
    with jax.named_scope("pairs"):
        lax.fori_loop(0, H // 2 - 1, pair_body, 0)
    with jax.named_scope("last_pair"):
        attend(H // 2 - 1)


def _tail_phase(wg_hbm, wu_hbm, wd_hbm, wr_ref, out_hbm, c_wo, x_v, xn_v, wo_v, ctx_v, idx_s, sems,
                wg_v, wu_v, wd_v, h_v, acc_v):
    c_wg = pltpu.make_async_copy(wg_hbm, wg_v, sems.at[6])
    c_wu = pltpu.make_async_copy(wu_hbm, wu_v, sems.at[7])
    c_wd = pltpu.make_async_copy(wd_hbm, wd_v, sems.at[8])
    c_wg.start()
    c_wu.start()
    c_wd.start()
    c_wo.wait()
    wr = wr_ref[...].astype(f32)

    def out_copy(start, size, sem):
        rows = pl.ds(start, size)
        return pltpu.make_async_copy(x_v.at[rows, :], out_hbm.at[rows, :], sems.at[sem])

    def project(start, RB):
        ctx = jnp.concatenate([ctx_v[pl.ds(hh * S + start, RB), :] for hh in range(H)], axis=1)
        acc_v[pl.ds(0, RB), :] = jnp.dot(ctx, wo_v[...], preferred_element_type=f32)

    sub8 = lax.broadcasted_iota(jnp.int32, (8, 128), 0)

    def epilogue(start, RB, top):
        rows = pl.ds(start, RB)
        a = acc_v[pl.ds(0, RB), :]
        h = (x_v[rows, :].astype(f32) + a.astype(bf16).astype(f32)).astype(bf16)
        hf = h.astype(f32)
        ln = _ln(hf).astype(bf16)
        lnf = ln.astype(f32)
        r = jnp.sum(lnf * wr, axis=1, keepdims=True).astype(bf16).astype(f32)
        xn_v[rows, :] = ln
        x_v[rows, :] = (hf + lnf).astype(bf16)
        h_v[rows, :] = h
        out_copy(start, RB, 9).start()
        m1, i1, m2, i2 = top
        for t in range(RB // 8):
            v = jnp.broadcast_to(r[t * 8:(t + 1) * 8], (8, 128))
            tok = sub8 + (start + t * 8)
            gt1 = v > m1
            gt2 = v > m2
            m2 = jnp.where(gt1, m1, jnp.where(gt2, v, m2))
            i2 = jnp.where(gt1, i1, jnp.where(gt2, tok, i2))
            m1 = jnp.where(gt1, v, m1)
            i1 = jnp.where(gt1, tok, i1)
        return m1, i1, m2, i2

    blocks = [(sum(RBS[:n]), RB) for n, RB in enumerate(RBS)]
    with jax.named_scope("out_proj"):
        ninf = jnp.full((8, 128), -jnp.inf, f32)
        zero = jnp.zeros((8, 128), jnp.int32)
        top = (ninf, zero, ninf, zero)
        project(*blocks[0])
        for n, blk in enumerate(blocks):
            top = epilogue(*blk, top)
            if n + 1 < len(blocks):
                project(*blocks[n + 1])

    r = jnp.concatenate([top[0], top[2]], axis=0)
    tok = jnp.concatenate([top[1], top[3]], axis=0)
    m1 = jnp.max(r, axis=0, keepdims=True)
    i1 = jnp.min(jnp.where(r == m1, tok, S - 1), axis=0, keepdims=True)
    r2 = jnp.where(tok == i1, -jnp.inf, r)
    m2 = jnp.max(r2, axis=0, keepdims=True)
    i2 = jnp.min(jnp.where(r2 == m2, tok, S - 1), axis=0, keepdims=True)
    idx_s[0] = jnp.max(i1)
    idx_s[1] = jnp.max(i2)
    m1 = m1[:, :1]
    m2 = m2[:, :1]
    t1 = idx_s[0]
    t2 = idx_s[1]
    b1 = pl.multiple_of((t1 // 16) * 16, 16)
    b2 = pl.multiple_of((t2 // 16) * 16, 16)
    sub = lax.broadcasted_iota(jnp.int32, (16, M), 0)
    sel1 = sub == (t1 - b1)
    sel2 = sub == (t2 - b2)
    ln1 = jnp.where(sel1, xn_v[pl.ds(b1, 16), :].astype(f32), 0.0)
    ln2 = jnp.where(sel2, xn_v[pl.ds(b2, 16), :].astype(f32), 0.0)
    x1 = jnp.sum(ln1, axis=0, keepdims=True)
    x2 = jnp.sum(ln2, axis=0, keepdims=True)
    xs = jnp.where(sub == 0, x1, jnp.where(sub == 1, x2, 0.0)).astype(bf16)

    c_wg.wait()
    c_wu.wait()
    g = jnp.dot(xs, wg_v[...], preferred_element_type=f32).astype(bf16).astype(f32)
    u = jnp.dot(xs, wu_v[...], preferred_element_type=f32).astype(bf16).astype(f32)
    sg = (g * (1.0 / (1.0 + jnp.exp(-g)))).astype(bf16).astype(f32)
    act = (sg * u).astype(bf16)
    with jax.named_scope("wait_wd"):
        c_wd.wait()
    y = jnp.dot(act, wd_v[...], preferred_element_type=f32).astype(bf16).astype(f32)
    g1 = (1.0 / (1.0 + jnp.exp(-m1))).astype(bf16).astype(f32)
    g2 = (1.0 / (1.0 + jnp.exp(-m2))).astype(bf16).astype(f32)
    y1 = (y[0:1, :] * g1).astype(bf16).astype(f32)
    y2 = (y[1:2, :] * g2).astype(bf16).astype(f32)

    with jax.named_scope("wait_out"):
        for blk in blocks:
            out_copy(*blk, 9).wait()
    for b, sel, yy in ((b1, sel1, y1), (b2, sel2, y2)):
        rows = pl.ds(b, 16)
        hrow = h_v[rows, :].astype(f32)
        lnrow = xn_v[rows, :].astype(f32)
        new = (hrow + (lnrow + yy).astype(bf16).astype(f32)).astype(bf16)
        x_v[rows, :] = jnp.where(sel, new, x_v[rows, :])

    out_copy(b1, 16, 9).start()

    @pl.when(b1 != b2)
    def _():
        c = out_copy(b2, 16, 0)
        c.start()
        c.wait()
    out_copy(b1, 16, 9).wait()


def _kernel(x_hbm, ckv_hbm, wq_hbm, wuk_hbm, wuv_hbm, wo_hbm, wr_ref, wg_hbm, wu_hbm, wd_hbm,
            out_hbm, x_v, xn_v, wo_v, ctx_v, idx_s, sems):
    c_wo = pltpu.make_async_copy(wo_hbm, wo_v, sems.at[5])
    pl.run_scoped(
        functools.partial(_attention_phase, x_hbm, ckv_hbm, wq_hbm, wuk_hbm, wuv_hbm, c_wo,
                          x_v, xn_v, ctx_v, sems),
        pltpu.VMEM((S, DC), bf16),
        pltpu.VMEM((H // 2, M, 2 * D), bf16), pltpu.VMEM((H // 2, DC, 2 * D), bf16),
        pltpu.VMEM((H // 2, DC, 2 * D), bf16),
        pltpu.VMEM((S, 2 * D), bf16), pltpu.VMEM((S, 2 * D), bf16), pltpu.VMEM((S, 2 * D), bf16))
    pl.run_scoped(
        functools.partial(_tail_phase, wg_hbm, wu_hbm, wd_hbm, wr_ref, out_hbm, c_wo,
                          x_v, xn_v, wo_v, ctx_v, idx_s, sems),
        pltpu.VMEM((M, F), bf16), pltpu.VMEM((M, F), bf16), pltpu.VMEM((F, M), bf16), pltpu.VMEM((S, M), bf16),
        pltpu.VMEM((max(RBS), M), f32))


@jax.jit
def pallas_sequential_preLN__compressed_kv_cla__moe_arch_mod__prompt_kernel(
    A_x, A_c_kv, A_w_q, A_w_uk, A_w_uv, A_w_o, B_x, B_w_r, B_w_gate, B_w_up, B_w_down,
):
    any_spec = pl.BlockSpec(memory_space=pl.ANY)
    vm = lambda shape, dt=bf16: pltpu.VMEM(shape, dt)
    out = pl.pallas_call(
        _kernel,
        out_shape=jax.ShapeDtypeStruct((S, M), bf16),
        in_specs=[any_spec] * 6 + [pl.BlockSpec(memory_space=pltpu.VMEM)] + [any_spec] * 3,
        out_specs=any_spec,
        scratch_shapes=[
            vm((S, M)), vm((S, M)), vm((H * D, M)), vm((S * H, D)),
            pltpu.SMEM((2,), jnp.int32),
            pltpu.SemaphoreType.DMA((10,)),
        ],
        compiler_params=pltpu.CompilerParams(vmem_limit_bytes=127 * 1024 * 1024),
    )(
        A_x.reshape(S, M), A_c_kv.reshape(S, DC),
        A_w_q.reshape(M * H, D), A_w_uk.reshape(DC * H, D), A_w_uv.reshape(DC * H, D),
        A_w_o.reshape(H * D, M), B_w_r.reshape(1, M), B_w_gate, B_w_up, B_w_down,
    )
    return out.reshape(1, S, M)
```

```python
import functools
import math

import numpy as np
import jax
import jax.numpy as jnp
from jax import lax
import jax.experimental.pallas as pl
import jax.experimental.pallas.tpu as pltpu

S = 2048
M = 1024
H = 32
D = 128
DC = 512
F = 3584
EPS = 1e-5
BQ = 256
LOOK = 2
DEP = False
PSTART = 15
PR = 2048
RBS = (1024, 512, 256, 256)
NEG = -1e30
QSCALE = float(D ** -0.5 * math.log2(math.e))

f32 = jnp.float32
bf16 = jnp.bfloat16
u32 = jnp.uint32


def _ln(x):
    m = jnp.mean(x, axis=-1, keepdims=True)
    xc = x - m
    v = jnp.mean(xc * xc, axis=-1, keepdims=True)
    return xc * lax.rsqrt(v + EPS)


def _unpack_pair(raw32, base, g4, o, rows):
    w = raw32.at[pl.ds(base + g4, rows * (H // 2) - 12), :][pl.ds(o, rows, stride=H // 2), :]
    lo = lax.bitcast_convert_type(w.astype(jnp.uint16), bf16)
    hi = lax.bitcast_convert_type((w >> 16).astype(jnp.uint16), bf16)
    return jnp.concatenate([lo, hi], axis=1)


def _softmax_rows(s):
    m = jnp.max(s, axis=1, keepdims=True)
    p = jnp.exp2(s - m)
    l = jnp.sum(p, axis=1, keepdims=True)
    rl = pl.reciprocal(l, approx=True)
    rl = rl * (2.0 - l * rl)
    return p.astype(bf16), rl


T = 128
NS = BQ // T


def _scores(q_ref, k_ref, a, i):
    lanes = pl.ds(a * D, D)
    k0 = i * BQ + T
    nt = (((1,), (1,)), ((), ()))
    q = q_ref[pl.ds(i * BQ, BQ), lanes]
    out = [lax.dot_general(q, k_ref[pl.ds(0, k0), lanes], nt, preferred_element_type=f32)]
    for t in range(1, NS):
        out.append(lax.dot_general(q[t * T:], k_ref[pl.ds(k0 + (t - 1) * T, T), lanes], nt,
                                   preferred_element_type=f32))
    return out


def _probs(sc, i):
    row = lax.broadcasted_iota(jnp.int32, (T, T), 0)
    col = lax.broadcasted_iota(jnp.int32, (T, T), 1)
    tri = col <= row
    k0 = i * BQ + T
    ps, rls = [], []
    for r in range(NS):
        parts = [sc[0][r * T:(r + 1) * T]] + [sc[t][(r - t) * T:(r - t + 1) * T] for t in range(1, r + 1)]
        s = jnp.concatenate(parts, axis=1) if len(parts) > 1 else parts[0]
        n = s.shape[1]
        sd = jnp.where(tri, s[:, n - T:], NEG)
        s = jnp.concatenate([s[:, :n - T], sd], axis=1) if n > T else sd
        p, rl = _softmax_rows(s)
        ps.append(p)
        rls.append(rl)
    pieces = [jnp.concatenate([p[:, :k0] for p in ps], axis=0) if NS > 1 else ps[0]]
    for t in range(1, NS):
        c = k0 + (t - 1) * T
        tiles = [ps[r][:, c:c + T] for r in range(t, NS)]
        pieces.append(jnp.concatenate(tiles, axis=0) if len(tiles) > 1 else tiles[0])
    return pieces, rls


def _context(pr, v_ref, ctx_ref, a, i, h0):
    pieces, rls = pr
    lanes = pl.ds(a * D, D)
    k0 = i * BQ + T
    o = jnp.dot(pieces[0], v_ref[pl.ds(0, k0), lanes], preferred_element_type=f32)
    strips = [o[r * T:(r + 1) * T] for r in range(NS)]
    for t in range(1, NS):
        ot = jnp.dot(pieces[t], v_ref[pl.ds(k0 + (t - 1) * T, T), lanes], preferred_element_type=f32)
        for r in range(t, NS):
            strips[r] = strips[r] + ot[(r - t) * T:(r - t + 1) * T]
    o = jnp.concatenate([strips[r] * rls[r] for r in range(NS)], axis=0)
    ctx_ref[pl.ds(pl.multiple_of((h0 + a) * S + i * BQ, BQ), BQ), :] = o.astype(bf16)


def _attention_phase(x_hbm, ckv_hbm, wq_hbm, wuk_hbm, wuv_hbm, c_wo, x_v, xn_v, ctx_v, sems,
                     ckv_v, wq_v, wk_v, wv_v, q_v, k_v, v_v):
    nq, nk = M * H, DC * H
    c_x = pltpu.make_async_copy(x_hbm, x_v, sems.at[0])
    c_ckv = pltpu.make_async_copy(ckv_hbm, ckv_v, sems.at[1])
    c_wq = pltpu.make_async_copy(wq_hbm, ctx_v.at[pl.ds(0, nq), :], sems.at[2])
    c_wuk = pltpu.make_async_copy(wuk_hbm, ctx_v.at[pl.ds(nq, nk), :], sems.at[3])
    c_wuv = pltpu.make_async_copy(wuv_hbm, ctx_v.at[pl.ds(nq + nk, nk), :], sems.at[4])
    raw32 = ctx_v.bitcast(u32)

    def unpack(dst, base, rows):
        def body(g, _):
            g4 = pl.multiple_of(g * 4, 4)
            for o in range(4):
                dst[g4 + o] = _unpack_pair(raw32, base, g4, o, rows)
            return 0
        lax.fori_loop(0, H // 8, body, 0)

    def proj_kv(j):
        ckv = ckv_v[...]
        k_v[...] = jnp.dot(ckv, wk_v[j], preferred_element_type=f32).astype(bf16)
        v_v[...] = jnp.dot(ckv, wv_v[j], preferred_element_type=f32).astype(bf16)

    def proj_q(j):
        q_v[...] = (jnp.dot(xn_v[...], wq_v[j], preferred_element_type=f32) * QSCALE).astype(bf16)

    def attend(j):
        blocks = [(i, a) for a in range(2) for i in reversed(range(S // BQ))]
        sc = [_scores(q_v, k_v, a, i) for i, a in blocks[:LOOK]]
        for n, (i, a) in enumerate(blocks):
            if n + LOOK < len(blocks):
                sc.append(_scores(q_v, k_v, blocks[n + LOOK][1], blocks[n + LOOK][0]))
            _context(_probs(sc.pop(0), i), v_v, ctx_v, a, i, 2 * j)

    c_wq.start()
    c_x.start()
    c_wuk.start()
    c_wuv.start()
    c_ckv.start()
    c_wo.start()

    def ln_body(i, _):
        rows = pl.ds(pl.multiple_of(i * 256, 256), 256)
        xn_v[rows, :] = _ln(x_v[rows, :].astype(f32)).astype(bf16)
        return 0
    with jax.named_scope("wait_q"):
        c_wq.wait()
    with jax.named_scope("unpack_q"):
        unpack(wq_v, 0, M)
    with jax.named_scope("wait_x"):
        c_x.wait()
    with jax.named_scope("ln"):
        lax.fori_loop(0, S // 256, ln_body, 0)
    with jax.named_scope("proj_q0"):
        proj_q(0)
    with jax.named_scope("wait_k"):
        c_wuk.wait()
    with jax.named_scope("unpack_k"):
        unpack(wk_v, nq // 2, DC)
    with jax.named_scope("wait_v"):
        c_wuv.wait()
    with jax.named_scope("unpack_v"):
        unpack(wv_v, (nq + nk) // 2, DC)
    with jax.named_scope("proj_kv0"):
        c_ckv.wait()
        proj_kv(0)

    def pair_body(j, _):
        attend(j)
        proj_kv(j + 1)
        proj_q(j + 1)
        return 0
    with jax.named_scope("pairs"):
        lax.fori_loop(0, H // 2 - 1, pair_body, 0)
    with jax.named_scope("last_pair"):
        attend(H // 2 - 1)


def _tail_phase(wg_hbm, wu_hbm, wd_hbm, wr_ref, out_hbm, c_wo, x_v, xn_v, wo_v, ctx_v, idx_s, sems,
                wg_v, wu_v, wd_v, h_v, acc_v):
    c_wg = pltpu.make_async_copy(wg_hbm, wg_v, sems.at[6])
    c_wu = pltpu.make_async_copy(wu_hbm, wu_v, sems.at[7])
    c_wd = pltpu.make_async_copy(wd_hbm, wd_v, sems.at[8])
    c_wg.start()
    c_wu.start()
    c_wd.start()
    c_wo.wait()
    wr = wr_ref[...].astype(f32).reshape(1, M)

    def out_copy(start, size, sem):
        rows = pl.ds(start, size)
        return pltpu.make_async_copy(x_v.at[rows, :], out_hbm.at[rows, :], sems.at[sem])

    def project(start, RB):
        ctx = jnp.concatenate([ctx_v[pl.ds(hh * S + start, RB), :] for hh in range(H)], axis=1)
        acc_v[pl.ds(0, RB), :] = jnp.dot(ctx, wo_v[...], preferred_element_type=f32)

    sub8 = lax.broadcasted_iota(jnp.int32, (8, 128), 0)

    def epilogue(start, RB, top):
        rows = pl.ds(start, RB)
        a = acc_v[pl.ds(0, RB), :]
        h = (x_v[rows, :].astype(f32) + a.astype(bf16).astype(f32)).astype(bf16)
        hf = h.astype(f32)
        ln = _ln(hf).astype(bf16)
        lnf = ln.astype(f32)
        r = jnp.sum(lnf * wr, axis=1, keepdims=True).astype(bf16).astype(f32)
        xn_v[rows, :] = ln
        x_v[rows, :] = (hf + lnf).astype(bf16)
        h_v[rows, :] = h
        out_copy(start, RB, 9).start()
        m1, i1, m2, i2 = top
        for t in range(RB // 8):
            v = jnp.broadcast_to(r[t * 8:(t + 1) * 8], (8, 128))
            tok = sub8 + (start + t * 8)
            gt1 = v > m1
            gt2 = v > m2
            m2 = jnp.where(gt1, m1, jnp.where(gt2, v, m2))
            i2 = jnp.where(gt1, i1, jnp.where(gt2, tok, i2))
            m1 = jnp.where(gt1, v, m1)
            i1 = jnp.where(gt1, tok, i1)
        return m1, i1, m2, i2

    blocks = [(sum(RBS[:n]), RB) for n, RB in enumerate(RBS)]
    with jax.named_scope("out_proj"):
        ninf = jnp.full((8, 128), -jnp.inf, f32)
        zero = jnp.zeros((8, 128), jnp.int32)
        top = (ninf, zero, ninf, zero)
        project(*blocks[0])
        for n, blk in enumerate(blocks):
            top = epilogue(*blk, top)
            if n + 1 < len(blocks):
                project(*blocks[n + 1])

    r = jnp.concatenate([top[0], top[2]], axis=0)
    tok = jnp.concatenate([top[1], top[3]], axis=0)
    m1 = jnp.max(r, axis=0, keepdims=True)
    i1 = jnp.min(jnp.where(r == m1, tok, S - 1), axis=0, keepdims=True)
    r2 = jnp.where(tok == i1, -jnp.inf, r)
    m2 = jnp.max(r2, axis=0, keepdims=True)
    i2 = jnp.min(jnp.where(r2 == m2, tok, S - 1), axis=0, keepdims=True)
    idx_s[0] = jnp.max(i1)
    idx_s[1] = jnp.max(i2)
    m1 = m1[:, :1]
    m2 = m2[:, :1]
    t1 = idx_s[0]
    t2 = idx_s[1]
    b1 = pl.multiple_of((t1 // 16) * 16, 16)
    b2 = pl.multiple_of((t2 // 16) * 16, 16)
    sub = lax.broadcasted_iota(jnp.int32, (16, M), 0)
    sel1 = sub == (t1 - b1)
    sel2 = sub == (t2 - b2)
    ln1 = jnp.where(sel1, xn_v[pl.ds(b1, 16), :].astype(f32), 0.0)
    ln2 = jnp.where(sel2, xn_v[pl.ds(b2, 16), :].astype(f32), 0.0)
    x1 = jnp.sum(ln1, axis=0, keepdims=True)
    x2 = jnp.sum(ln2, axis=0, keepdims=True)
    xs = jnp.where(sub == 0, x1, jnp.where(sub == 1, x2, 0.0)).astype(bf16)

    c_wg.wait()
    c_wu.wait()
    g = jnp.dot(xs, wg_v[...], preferred_element_type=f32).astype(bf16).astype(f32)
    u = jnp.dot(xs, wu_v[...], preferred_element_type=f32).astype(bf16).astype(f32)
    sg = (g * (1.0 / (1.0 + jnp.exp(-g)))).astype(bf16).astype(f32)
    act = (sg * u).astype(bf16)
    with jax.named_scope("wait_wd"):
        c_wd.wait()
    y = sum(jnp.dot(act[:, k:k + 128], wd_v[pl.ds(k, 128), :], preferred_element_type=f32)
            for k in range(0, F, 128)).astype(bf16).astype(f32)
    g1 = (1.0 / (1.0 + jnp.exp(-m1))).astype(bf16).astype(f32)
    g2 = (1.0 / (1.0 + jnp.exp(-m2))).astype(bf16).astype(f32)
    y1 = (y[0:1, :] * g1).astype(bf16).astype(f32)
    y2 = (y[1:2, :] * g2).astype(bf16).astype(f32)

    with jax.named_scope("wait_out"):
        for blk in blocks:
            out_copy(*blk, 9).wait()
    for b, sel, yy in ((b1, sel1, y1), (b2, sel2, y2)):
        rows = pl.ds(b, 16)
        hrow = h_v[rows, :].astype(f32)
        lnrow = xn_v[rows, :].astype(f32)
        new = (hrow + (lnrow + yy).astype(bf16).astype(f32)).astype(bf16)
        x_v[rows, :] = jnp.where(sel, new, x_v[rows, :])

    out_copy(b1, 16, 9).start()

    @pl.when(b1 != b2)
    def _():
        c = out_copy(b2, 16, 0)
        c.start()
        c.wait()
    out_copy(b1, 16, 9).wait()


def _kernel(x_hbm, ckv_hbm, wq_hbm, wuk_hbm, wuv_hbm, wo_hbm, wr_ref, wg_hbm, wu_hbm, wd_hbm,
            out_hbm, x_v, xn_v, wo_v, ctx_v, idx_s, sems):
    c_wo = pltpu.make_async_copy(wo_hbm, wo_v, sems.at[5])
    pl.run_scoped(
        functools.partial(_attention_phase, x_hbm, ckv_hbm, wq_hbm, wuk_hbm, wuv_hbm, c_wo,
                          x_v, xn_v, ctx_v, sems),
        pltpu.VMEM((S, DC), bf16),
        pltpu.VMEM((H // 2, M, 2 * D), bf16), pltpu.VMEM((H // 2, DC, 2 * D), bf16),
        pltpu.VMEM((H // 2, DC, 2 * D), bf16),
        pltpu.VMEM((S, 2 * D), bf16), pltpu.VMEM((S, 2 * D), bf16), pltpu.VMEM((S, 2 * D), bf16))
    pl.run_scoped(
        functools.partial(_tail_phase, wg_hbm, wu_hbm, wd_hbm, wr_ref, out_hbm, c_wo,
                          x_v, xn_v, wo_v, ctx_v, idx_s, sems),
        pltpu.VMEM((M, F), bf16), pltpu.VMEM((M, F), bf16), pltpu.VMEM((F, M), bf16), pltpu.VMEM((S, M), bf16),
        pltpu.VMEM((max(RBS), M), f32))


@jax.jit
def pallas_sequential_preLN__compressed_kv_cla__moe_arch_mod__prompt_kernel(
    A_x, A_c_kv, A_w_q, A_w_uk, A_w_uv, A_w_o, B_x, B_w_r, B_w_gate, B_w_up, B_w_down,
):
    any_spec = pl.BlockSpec(memory_space=pl.ANY)
    vm = lambda shape, dt=bf16: pltpu.VMEM(shape, dt)
    out = pl.pallas_call(
        _kernel,
        out_shape=jax.ShapeDtypeStruct((S, M), bf16),
        in_specs=[any_spec] * 6 + [pl.BlockSpec(memory_space=pltpu.VMEM)] + [any_spec] * 3,
        out_specs=any_spec,
        scratch_shapes=[
            vm((S, M)), vm((S, M)), vm((H * D, M)), vm((S * H, D)),
            pltpu.SMEM((2,), jnp.int32),
            pltpu.SemaphoreType.DMA((10,)),
        ],
        compiler_params=pltpu.CompilerParams(vmem_limit_bytes=127 * 1024 * 1024),
    )(
        A_x.reshape(S, M), A_c_kv.reshape(S, DC),
        A_w_q.reshape(M * H, D), A_w_uk.reshape(DC * H, D), A_w_uv.reshape(DC * H, D),
        A_w_o.reshape(H * D, M), B_w_r, B_w_gate, B_w_up, B_w_down,
    )
    return out.reshape(1, S, M)
```

```python
import functools
import math

import numpy as np
import jax
import jax.numpy as jnp
from jax import lax
import jax.experimental.pallas as pl
import jax.experimental.pallas.tpu as pltpu

S = 2048
M = 1024
H = 32
D = 128
DC = 512
F = 3584
EPS = 1e-5
BQ = 256
UC = 128
LOOK = 2
DEP = False
PSTART = 15
PR = 2048
RBS = (256,) * 8
NEG = -1e30
QSCALE = float(D ** -0.5 * math.log2(math.e))

f32 = jnp.float32
bf16 = jnp.bfloat16
u32 = jnp.uint32


def _ln(x):
    m = jnp.mean(x, axis=-1, keepdims=True)
    xc = x - m
    v = jnp.mean(xc * xc, axis=-1, keepdims=True)
    return xc * lax.rsqrt(v + EPS)


def _softmax_rows(s):
    m = jnp.max(s, axis=1, keepdims=True)
    p = jnp.exp2(s - m)
    l = jnp.sum(p, axis=1, keepdims=True)
    rl = pl.reciprocal(l, approx=True)
    rl = rl * (2.0 - l * rl)
    return p.astype(bf16), rl


T = 128
NS = BQ // T


def _scores(q_ref, k_ref, a, i):
    lanes = pl.ds(a * D, D)
    k0 = i * BQ + T
    nt = (((1,), (1,)), ((), ()))
    q = q_ref[pl.ds(i * BQ, BQ), lanes]
    out = [lax.dot_general(q, k_ref[pl.ds(0, k0), lanes], nt, preferred_element_type=f32)]
    for t in range(1, NS):
        out.append(lax.dot_general(q[t * T:], k_ref[pl.ds(k0 + (t - 1) * T, T), lanes], nt,
                                   preferred_element_type=f32))
    return out


def _probs(sc, i):
    row = lax.broadcasted_iota(jnp.int32, (T, T), 0)
    col = lax.broadcasted_iota(jnp.int32, (T, T), 1)
    tri = col <= row
    k0 = i * BQ + T
    ps, rls = [], []
    for r in range(NS):
        parts = [sc[0][r * T:(r + 1) * T]] + [sc[t][(r - t) * T:(r - t + 1) * T] for t in range(1, r + 1)]
        s = jnp.concatenate(parts, axis=1) if len(parts) > 1 else parts[0]
        n = s.shape[1]
        sd = jnp.where(tri, s[:, n - T:], NEG)
        s = jnp.concatenate([s[:, :n - T], sd], axis=1) if n > T else sd
        p, rl = _softmax_rows(s)
        ps.append(p)
        rls.append(rl)
    pieces = [jnp.concatenate([p[:, :k0] for p in ps], axis=0) if NS > 1 else ps[0]]
    for t in range(1, NS):
        c = k0 + (t - 1) * T
        tiles = [ps[r][:, c:c + T] for r in range(t, NS)]
        pieces.append(jnp.concatenate(tiles, axis=0) if len(tiles) > 1 else tiles[0])
    return pieces, rls


def _context(pr, v_ref, ctx_ref, a, i, h0):
    pieces, rls = pr
    lanes = pl.ds(a * D, D)
    k0 = i * BQ + T
    o = jnp.dot(pieces[0], v_ref[pl.ds(0, k0), lanes], preferred_element_type=f32)
    strips = [o[r * T:(r + 1) * T] for r in range(NS)]
    for t in range(1, NS):
        ot = jnp.dot(pieces[t], v_ref[pl.ds(k0 + (t - 1) * T, T), lanes], preferred_element_type=f32)
        for r in range(t, NS):
            strips[r] = strips[r] + ot[(r - t) * T:(r - t + 1) * T]
    o = jnp.concatenate([strips[r] * rls[r] for r in range(NS)], axis=0)
    ctx_ref[pl.ds(pl.multiple_of((h0 + a) * S + i * BQ, BQ), BQ), :] = o.astype(bf16)


def _attention_phase(x_hbm, ckv_hbm, wq_hbm, wuk_hbm, wuv_hbm, c_wo, x_v, xn_v, ctx_v, sems,
                     ckv_v, wq_raw, wk_raw, wv_raw, tmp_v, wq_v, wk_v, wv_v, q_v, k_v, v_v):
    HH = H // 2
    c_x = pltpu.make_async_copy(x_hbm, x_v, sems.at[0])
    c_ckv = pltpu.make_async_copy(ckv_hbm, ckv_v, sems.at[1])

    def w_copy(n, hf):
        src, dst = ((wq_hbm, wq_raw), (wuk_hbm, wk_raw), (wuv_hbm, wv_raw))[n]
        return pltpu.make_async_copy(src.at[:, pl.ds(hf * HH, HH), :], dst.at[hf],
                                     sems.at[(2, 10)[hf] + n])

    def unpack_rows(raw, dst, hf, r0, rows):
        w = raw[hf, pl.ds(r0, rows)].reshape(rows * HH, D)
        tmp_v[pl.ds(0, rows * HH // 2), :] = pltpu.bitcast(w, u32)
        for o in range(HH // 2):
            w = tmp_v[pl.ds(o, rows, stride=HH // 2), :]
            lo = lax.bitcast_convert_type(w.astype(jnp.uint16), bf16)
            hi = lax.bitcast_convert_type((w >> 16).astype(jnp.uint16), bf16)
            dst[hf * (HH // 2) + o, pl.ds(r0, rows), :] = jnp.concatenate([lo, hi], axis=1)

    def unpack(raw, dst, hf, r0, rows):
        def body(c, _):
            unpack_rows(raw, dst, hf, pl.multiple_of(c * UC, UC), UC)
            return 0
        lax.fori_loop(0, rows // UC, body, 0)

    def proj_kv(j):
        ckv = ckv_v[...]
        k_v[...] = jnp.dot(ckv, wk_v[j], preferred_element_type=f32).astype(bf16)
        v_v[...] = jnp.dot(ckv, wv_v[j], preferred_element_type=f32).astype(bf16)

    def proj_q(j):
        q_v[...] = (jnp.dot(xn_v[...], wq_v[j], preferred_element_type=f32) * QSCALE).astype(bf16)

    def attend(j):
        blocks = [(i, a) for i in reversed(range(S // BQ)) for a in range(2)]
        sc = [_scores(q_v, k_v, a, i) for i, a in blocks[:LOOK]]
        for n, (i, a) in enumerate(blocks):
            if n + LOOK < len(blocks):
                sc.append(_scores(q_v, k_v, blocks[n + LOOK][1], blocks[n + LOOK][0]))
            _context(_probs(sc.pop(0), i), v_v, ctx_v, a, i, 2 * j)

    c_x.start()
    w_copy(0, 0).start()
    w_copy(1, 0).start()
    w_copy(2, 0).start()
    c_ckv.start()
    for n in range(3):
        w_copy(n, 1).start()
    c_wo.start()

    def ln_body(i, _):
        rows = pl.ds(pl.multiple_of(i * 256, 256), 256)
        xn_v[rows, :] = _ln(x_v[rows, :].astype(f32)).astype(bf16)
        return 0
    with jax.named_scope("wait_x"):
        c_x.wait()
    with jax.named_scope("ln"):
        lax.fori_loop(0, S // 256, ln_body, 0)
    with jax.named_scope("wait_q"):
        w_copy(0, 0).wait()
    with jax.named_scope("unpack_q"):
        unpack(wq_raw, wq_v, 0, 0, M)
    with jax.named_scope("proj_q0"):
        proj_q(0)
    with jax.named_scope("wait_k"):
        w_copy(1, 0).wait()
    with jax.named_scope("unpack_k"):
        unpack(wk_raw, wk_v, 0, 0, DC)
    with jax.named_scope("wait_v"):
        w_copy(2, 0).wait()
    with jax.named_scope("unpack_v"):
        unpack(wv_raw, wv_v, 0, 0, DC)
    with jax.named_scope("proj_kv0"):
        c_ckv.wait()
        proj_kv(0)

    with jax.named_scope("unpack_2"):
        for n, (raw, dst, rows) in enumerate(((wq_raw, wq_v, M), (wk_raw, wk_v, DC), (wv_raw, wv_v, DC))):
            w_copy(n, 1).wait()
            unpack(raw, dst, 1, 0, rows)

    def pair_body(j, _):
        attend(j)
        proj_kv(j + 1)
        proj_q(j + 1)
        return 0
    with jax.named_scope("pairs"):
        lax.fori_loop(0, H // 2 - 1, pair_body, 0)
    with jax.named_scope("last_pair"):
        attend(H // 2 - 1)


def _tail_phase(wg_hbm, wu_hbm, wd_hbm, wr_ref, out_hbm, c_wo, x_v, xn_v, wo_v, ctx_v, idx_s, sems,
                wg_v, wu_v, wd_v, h_v, acc_v):
    c_wg = pltpu.make_async_copy(wg_hbm, wg_v, sems.at[6])
    c_wu = pltpu.make_async_copy(wu_hbm, wu_v, sems.at[7])
    c_wd = pltpu.make_async_copy(wd_hbm, wd_v, sems.at[8])
    c_wg.start()
    c_wu.start()
    c_wd.start()
    c_wo.wait()
    wr = wr_ref[...].astype(f32).reshape(1, M)

    def out_copy(start, size, sem):
        rows = pl.ds(start, size)
        return pltpu.make_async_copy(x_v.at[rows, :], out_hbm.at[rows, :], sems.at[sem])

    def project(start, RB):
        ctx = jnp.concatenate([ctx_v[pl.ds(hh * S + start, RB), :] for hh in range(H)], axis=1)
        acc_v[pl.ds(0, RB), :] = jnp.dot(ctx, wo_v[...], preferred_element_type=f32)

    sub8 = lax.broadcasted_iota(jnp.int32, (8, 128), 0)

    def epilogue(start, RB, top):
        rows = pl.ds(start, RB)
        a = acc_v[pl.ds(0, RB), :]
        h = (x_v[rows, :].astype(f32) + a.astype(bf16).astype(f32)).astype(bf16)
        hf = h.astype(f32)
        ln = _ln(hf).astype(bf16)
        lnf = ln.astype(f32)
        r = jnp.sum(lnf * wr, axis=1, keepdims=True).astype(bf16).astype(f32)
        xn_v[rows, :] = ln
        x_v[rows, :] = (hf + lnf).astype(bf16)
        h_v[rows, :] = h
        out_copy(start, RB, 9).start()
        m1, i1, m2, i2 = top
        for t in range(RB // 8):
            v = jnp.broadcast_to(r[t * 8:(t + 1) * 8], (8, 128))
            tok = sub8 + (start + t * 8)
            gt1 = v > m1
            gt2 = v > m2
            m2 = jnp.where(gt1, m1, jnp.where(gt2, v, m2))
            i2 = jnp.where(gt1, i1, jnp.where(gt2, tok, i2))
            m1 = jnp.where(gt1, v, m1)
            i1 = jnp.where(gt1, tok, i1)
        return m1, i1, m2, i2

    blocks = [(sum(RBS[:n]), RB) for n, RB in enumerate(RBS)]
    with jax.named_scope("out_proj"):
        ninf = jnp.full((8, 128), -jnp.inf, f32)
        zero = jnp.zeros((8, 128), jnp.int32)
        top = (ninf, zero, ninf, zero)
        project(*blocks[0])
        for n, blk in enumerate(blocks):
            top = epilogue(*blk, top)
            if n + 1 < len(blocks):
                project(*blocks[n + 1])

    r = jnp.concatenate([top[0], top[2]], axis=0)
    tok = jnp.concatenate([top[1], top[3]], axis=0)
    m1 = jnp.max(r, axis=0, keepdims=True)
    i1 = jnp.min(jnp.where(r == m1, tok, S - 1), axis=0, keepdims=True)
    r2 = jnp.where(tok == i1, -jnp.inf, r)
    m2 = jnp.max(r2, axis=0, keepdims=True)
    i2 = jnp.min(jnp.where(r2 == m2, tok, S - 1), axis=0, keepdims=True)
    idx_s[0] = jnp.max(i1)
    idx_s[1] = jnp.max(i2)
    m1 = m1[:, :1]
    m2 = m2[:, :1]
    t1 = idx_s[0]
    t2 = idx_s[1]
    b1 = pl.multiple_of((t1 // 16) * 16, 16)
    b2 = pl.multiple_of((t2 // 16) * 16, 16)
    sub = lax.broadcasted_iota(jnp.int32, (16, M), 0)
    sel1 = sub == (t1 - b1)
    sel2 = sub == (t2 - b2)
    ln1 = jnp.where(sel1, xn_v[pl.ds(b1, 16), :].astype(f32), 0.0)
    ln2 = jnp.where(sel2, xn_v[pl.ds(b2, 16), :].astype(f32), 0.0)
    x1 = jnp.sum(ln1, axis=0, keepdims=True)
    x2 = jnp.sum(ln2, axis=0, keepdims=True)
    xs = jnp.where(sub == 0, x1, jnp.where(sub == 1, x2, 0.0)).astype(bf16)

    c_wg.wait()
    c_wu.wait()
    g = jnp.dot(xs, wg_v[...], preferred_element_type=f32).astype(bf16).astype(f32)
    u = jnp.dot(xs, wu_v[...], preferred_element_type=f32).astype(bf16).astype(f32)
    sg = (g * (1.0 / (1.0 + jnp.exp(-g)))).astype(bf16).astype(f32)
    act = (sg * u).astype(bf16)
    with jax.named_scope("wait_wd"):
        c_wd.wait()
    y = sum(jnp.dot(act[:, k:k + 128], wd_v[pl.ds(k, 128), :], preferred_element_type=f32)
            for k in range(0, F, 128)).astype(bf16).astype(f32)
    g1 = (1.0 / (1.0 + jnp.exp(-m1))).astype(bf16).astype(f32)
    g2 = (1.0 / (1.0 + jnp.exp(-m2))).astype(bf16).astype(f32)
    y1 = (y[0:1, :] * g1).astype(bf16).astype(f32)
    y2 = (y[1:2, :] * g2).astype(bf16).astype(f32)

    with jax.named_scope("wait_out"):
        for blk in blocks:
            out_copy(*blk, 9).wait()
    for b, sel, yy in ((b1, sel1, y1), (b2, sel2, y2)):
        rows = pl.ds(b, 16)
        hrow = h_v[rows, :].astype(f32)
        lnrow = xn_v[rows, :].astype(f32)
        new = (hrow + (lnrow + yy).astype(bf16).astype(f32)).astype(bf16)
        x_v[rows, :] = jnp.where(sel, new, x_v[rows, :])

    out_copy(b1, 16, 9).start()

    @pl.when(b1 != b2)
    def _():
        c = out_copy(b2, 16, 0)
        c.start()
        c.wait()
    out_copy(b1, 16, 9).wait()


def _kernel(x_hbm, ckv_hbm, wq_hbm, wuk_hbm, wuv_hbm, wo_hbm, wr_ref, wg_hbm, wu_hbm, wd_hbm,
            out_hbm, x_v, xn_v, wo_v, ctx_v, idx_s, sems):
    c_wo = pltpu.make_async_copy(wo_hbm, wo_v, sems.at[5])
    pl.run_scoped(
        functools.partial(_attention_phase, x_hbm, ckv_hbm, wq_hbm, wuk_hbm, wuv_hbm, c_wo,
                          x_v, xn_v, ctx_v, sems),
        pltpu.VMEM((S, DC), bf16),
        pltpu.VMEM((2, M, H // 2, D), bf16), pltpu.VMEM((2, DC, H // 2, D), bf16),
        pltpu.VMEM((2, DC, H // 2, D), bf16), pltpu.VMEM((M * H // 4 + 8, D), u32),
        pltpu.VMEM((H // 2, M, 2 * D), bf16), pltpu.VMEM((H // 2, DC, 2 * D), bf16),
        pltpu.VMEM((H // 2, DC, 2 * D), bf16),
        pltpu.VMEM((S, 2 * D), bf16), pltpu.VMEM((S, 2 * D), bf16), pltpu.VMEM((S, 2 * D), bf16))
    pl.run_scoped(
        functools.partial(_tail_phase, wg_hbm, wu_hbm, wd_hbm, wr_ref, out_hbm, c_wo,
                          x_v, xn_v, wo_v, ctx_v, idx_s, sems),
        pltpu.VMEM((M, F), bf16), pltpu.VMEM((M, F), bf16), pltpu.VMEM((F, M), bf16), pltpu.VMEM((S, M), bf16),
        pltpu.VMEM((max(RBS), M), f32))


@jax.jit
def pallas_sequential_preLN__compressed_kv_cla__moe_arch_mod__prompt_kernel(
    A_x, A_c_kv, A_w_q, A_w_uk, A_w_uv, A_w_o, B_x, B_w_r, B_w_gate, B_w_up, B_w_down,
):
    any_spec = pl.BlockSpec(memory_space=pl.ANY)
    vm = lambda shape, dt=bf16: pltpu.VMEM(shape, dt)
    out = pl.pallas_call(
        _kernel,
        out_shape=jax.ShapeDtypeStruct((S, M), bf16),
        in_specs=[any_spec] * 6 + [pl.BlockSpec(memory_space=pltpu.VMEM)] + [any_spec] * 3,
        out_specs=any_spec,
        scratch_shapes=[
            vm((S, M)), vm((S, M)), vm((H * D, M)), vm((S * H, D)),
            pltpu.SMEM((2,), jnp.int32),
            pltpu.SemaphoreType.DMA((13,)),
        ],
        compiler_params=pltpu.CompilerParams(vmem_limit_bytes=127 * 1024 * 1024),
    )(
        A_x.reshape(S, M), A_c_kv.reshape(S, DC),
        A_w_q, A_w_uk, A_w_uv,
        A_w_o.reshape(H * D, M), B_w_r, B_w_gate, B_w_up, B_w_down,
    )
    return out.reshape(1, S, M)
```
